```python
import jax
import jax.numpy as jnp

def _softmax(x, axis=-1):
    return jax.nn.softmax(x, axis=axis)
def _gelu(x):
    return jax.nn.gelu(x, approximate=True)
def _silu(x):
    return jax.nn.silu(x)
def _sigmoid(x):
    return jax.nn.sigmoid(x)
def _layernorm(x, axis=-1, eps=1e-5):
    m = jnp.mean(x, axis=axis, keepdims=True)
    v = jnp.var(x, axis=axis, keepdims=True)
    return (x - m) / jnp.sqrt(v + eps)
def _scatter_add(tgt, idx, src, axis=0):
    return tgt.at[idx].add(src)
def _segment_sum(src, seg, n):
    return jax.ops.segment_sum(src, seg, n)
class _Rng:
    def __init__(self, key):
        self._k = key
    def _next(self):
        self._k, sub = jax.random.split(self._k)
        return sub
    def normal(self, shape):
        return jax.random.normal(self._next(), shape, dtype=jnp.bfloat16)
    def randint(self, lo, hi, shape):
        return jax.random.randint(self._next(), shape, lo, hi, dtype=jnp.int32)
    def uniform(self, shape, lo=0.0, hi=1.0):
        return jax.random.uniform(self._next(), shape, jnp.bfloat16, lo, hi)
    def permutation(self, n):
        return jax.random.permutation(self._next(), n)


kernel_name = 'sequential_preLN__sliding_local_dilated__moe_arch_mod__prompt'

def setup_inputs():
    _rng = _Rng(jax.random.key(int.from_bytes(__import__("os").urandom(4), "little")))
    _w = (lambda a: (lambda t: t.astype(jnp.bfloat16) if jnp.issubdtype(t.dtype, jnp.floating) else t)(jnp.asarray(a)))
    def _A_setup():
        B, S, D = 1, 2048, 640
        return {
            "x": _w((lambda *s: _rng.normal(s) * 0.05)(B, S, D)),
            "wqkv": _w((lambda *s: _rng.normal(s) * 0.05)(D, 3 * D)),
            "wo": _w((lambda *s: _rng.normal(s) * 0.05)(D, D)),
        }
    _A_in = _A_setup()

    def _B_setup():
        B, S, D, F, C = 1, 2048, 640, 1536, 1
        return {
            "x": _w((lambda *s: _rng.normal(s) * 0.05)(B, S, D)),
            "w_r": _w((lambda *s: _rng.normal(s) * 0.05)(D)),
            "w_gate": _w((lambda *s: _rng.normal(s) * 0.05)(D, F)),
            "w_up": _w((lambda *s: _rng.normal(s) * 0.05)(D, F)),
            "w_down": _w((lambda *s: _rng.normal(s) * 0.05)(F, D)),
        }
    _B_in = _B_setup()

    return {
        "A_x": _A_in["x"],
        "A_wqkv": _A_in["wqkv"],
        "A_wo": _A_in["wo"],
        "B_x": _B_in["x"],
        "B_w_r": _B_in["w_r"],
        "B_w_gate": _B_in["w_gate"],
        "B_w_up": _B_in["w_up"],
        "B_w_down": _B_in["w_down"],
    }

def reference(A_x, A_wqkv, A_wo, B_x, B_w_r, B_w_gate, B_w_up, B_w_down):
    def _A_ref(x, wqkv, wo):
        B, S, D = x.shape
        H = 32; Dh = D // H
        W, dil = 8, 2
        qkv = (lambda x, *d: x.transpose(*d))((x @ wqkv).reshape(B, S, 3, H, Dh), 2, 0, 3, 1, 4)
        q, k, v = qkv[0], qkv[1], qkv[2]
        scale = Dh ** -0.5
        pos = jnp.arange(S)
        off = jnp.arange(W) * dil
        idx = pos[:, None] - off[None, :]
        mask = idx >= 0
        idx_c = jnp.where(mask, idx, 0).reshape(-1)
        kg = k[:, :, idx_c, :].reshape(B, H, S, W, Dh)
        vg = v[:, :, idx_c, :].reshape(B, H, S, W, Dh)
        logits = jnp.einsum("bhsd,bhswd->bhsw", q, kg) * scale
        logits = jnp.where(mask[None, None, :, :], logits, -1e9)
        attn = _softmax(logits, axis=-1)
        o = jnp.einsum("bhsw,bhswd->bhsd", attn, vg)
        return (lambda x, *d: x.transpose(*d))(o, 0, 2, 1, 3).reshape(B, S, D) @ wo

    def _B_ref(x, w_r, w_gate, w_up, w_down):
        B, S, D = x.shape
        C = 1
        r = x @ w_r
        idx = jnp.argsort(-r, axis=-1)[:, :C]
        idx_e = jnp.repeat(idx.reshape(B, C, 1), D, axis=2)
        x_sel = jnp.take_along_axis(x, idx_e, axis=1)
        g = _silu(x_sel @ w_gate)
        u = x_sel @ w_up
        y = (g * u) @ w_down
        r_sel = _sigmoid(jnp.take_along_axis(r, idx, axis=1))
        y = y * r_sel.reshape(B, C, 1)
        b_off = (jnp.arange(B) * S).reshape(B, 1)
        flat_idx = (idx + b_off).reshape(B * C)
        zero = (x * 0.0).reshape(B * S, D)
        upd = _scatter_add(zero, flat_idx, y.reshape(B * C, D), axis=0)
        return x + upd.reshape(B, S, D)

    x = A_x
    h = x + _A_ref(_layernorm(x, axis=-1), A_wqkv, A_wo)
    h2 = h + _B_ref(_layernorm(h, axis=-1), B_w_r, B_w_gate, B_w_up, B_w_down)
    return h2
```

```python
import functools, os, contextlib
import jax, jax.numpy as jnp, numpy as np
from jax import lax
from jax.experimental import pallas as pl
from jax.experimental.pallas import tpu as pltpu

S, D, H, DH, W, DIL, F = 2048, 640, 32, 20, 8, 2, 1536
NP = D // 128
HALO = 16
T = int(os.environ.get('KT', 256))
NB = S // T
NIT = (NB - 4) // 2
BSUB = int(os.environ.get('BSUB', 128))
SUB = int(os.environ.get('KSUB', 128))
EPS = 1e-5
LOG2E = 1.4426950408889634
QSCALE = DH ** -0.5 * LOG2E
NEG = -1e9 * LOG2E
f32, bf16, u32, i32 = jnp.float32, jnp.bfloat16, jnp.uint32, jnp.int32


def SC(name):
    return jax.named_scope('SC_' + name) if os.environ.get('USE_SC') else contextlib.nullcontext()


def _ln(x):
    m = jnp.mean(x, axis=-1, keepdims=True)
    xc = x - m
    v = jnp.mean(xc * xc, axis=-1, keepdims=True)
    return xc * lax.rsqrt(v + EPS)


def _gather_rows(src, dst, dst_base, dst_col, scale=None):
    hi_mask = jnp.uint32(0xFFFF0000)
    for jp in range(NP):
        for ddl in range(2):
            dd = 2 * jp + ddl
            a = src[pl.ds(dd, 16, stride=20), :]
            b = src[pl.ds(dd + 10, 16, stride=20), :]
            if scale is None:
                lo = (a & 0xFFFF) | (b << 16)
                hi = (a >> 16) | (b & hi_mask)
            else:
                cast = lambda z: lax.bitcast_convert_type(z, f32) * scale
                lo = pltpu.pack_elementwise([cast(a << 16), cast(b << 16)], packed_dtype=bf16)
                hi = pltpu.pack_elementwise([cast(a & hi_mask), cast(b & hi_mask)], packed_dtype=bf16)
            r = dst_base + 64 * jp + 32 * ddl
            dst[r:r + 16, dst_col:dst_col + 128] = lo
            dst[r + 16:r + 32, dst_col:dst_col + 128] = hi


def kernel(x_hbm, wqkv_hbm, wo_hbm, wr_hbm, wg_hbm, wu_hbm, wd_hbm, out_hbm,
           xbuf, wraw, woraw, wt, wp, wop,
           xn0, xn1, qb0, qb1, kb0, kb1, vb0, vb1, ob0, ob1, hb0, hb1,
           hnb, outbuf, wr, wg, wu, wd,
           sem_x, sem_w, sem_o, sem_s, sem_r):
    xn, qb, kb, vb, ob, hb = (xn0, xn1), (qb0, qb1), (kb0, kb1), (vb0, vb1), (ob0, ob1), (hb0, hb1)

    def xcopy(i):
        return pltpu.make_async_copy(x_hbm.at[0, pl.ds(i * T, T), :], xbuf.at[pl.ds(i * T, T), :], sem_x.at[i])

    def ocopy(i):
        return pltpu.make_async_copy(outbuf.at[pl.ds(i * T, T), :], out_hbm.at[0, pl.ds(i * T, T), :], sem_o.at[i])

    def wcopy(m):
        return pltpu.make_async_copy(wqkv_hbm.at[:, pl.ds(m * D, D)], wraw.at[m], sem_w.at[m])

    cp_wo = pltpu.make_async_copy(wo_hbm, woraw, sem_s.at[0])
    cp_wr = pltpu.make_async_copy(wr_hbm, wr, sem_s.at[1])
    cp_wg = pltpu.make_async_copy(wg_hbm, wg, sem_s.at[2])
    cp_wu = pltpu.make_async_copy(wu_hbm, wu, sem_s.at[3])
    cp_wd = pltpu.make_async_copy(wd_hbm, wd, sem_s.at[4])

    def ordered_start(*cps):
        for cp in cps:
            cp.start()
            pl.semaphore_signal(sem_r, 1)
            pl.semaphore_wait(sem_r, 1)

    ordered_start(wcopy(0), xcopy(0), xcopy(1), wcopy(1), wcopy(2), cp_wo, cp_wr, xcopy(2))

    def row0(i):
        if isinstance(i, int):
            return i * T
        return pl.multiple_of(i * T, T)

    def half0(i):
        if isinstance(i, int):
            return i * (T // 2)
        return pl.multiple_of(i * (T // 2), T // 2)

    def transpose_chunk(m, kt):
        slab = wraw[m, kt * 128:(kt + 1) * 128, :]
        wt[kt] = pltpu.bitcast(slab.T, u32)

    def gather_w(m):
        for kt in range(NP):
            _gather_rows(wt.at[kt], wp, 320 * m, kt * 128, QSCALE if m == 0 else None)

    def prep_w(m):
        for kt in range(NP):
            transpose_chunk(m, kt)
        gather_w(m)

    def prep_wo():
        for nt in range(NP):
            wt[nt] = pltpu.bitcast(woraw[:, nt * 128:(nt + 1) * 128], u32)
        for nt in range(NP):
            _gather_rows(wt.at[nt], wop, 0, nt * 128)

    def stage_a(i, p):
        r0 = row0(i)
        for c in range(T // 16):
            x = xbuf[pl.ds(r0 + 16 * c, 16), :].astype(f32)
            xn[p][8 * c:8 * c + 8, :] = pltpu.bitcast(_ln(x).astype(bf16), u32)

    def halo(p):
        for j in range(NP):
            kb[p][j, 0:HALO, :] = kb[1 - p][j, T:T + HALO, :]
            vb[p][j, 0:HALO, :] = vb[1 - p][j, T:T + HALO, :]

    def stage_b(p, ms=(0, 1, 2), lo=0, hi=T):
        xv = pltpu.bitcast(xn[p][lo // 2:hi // 2, :], bf16)
        for m in ms:
            dst = (qb[p], kb[p], vb[p])[m]
            off = 0 if m == 0 else HALO
            wm = pltpu.bitcast(wp[320 * m:320 * (m + 1), :], bf16)
            r = lax.dot_general(xv, wm, (((1,), (1,)), ((), ())), preferred_element_type=f32)
            for j in range(NP):
                dst[j, off + lo:off + hi, :] = r[:, j * 128:(j + 1) * 128]

    def stage_c(i, p, lo=0, hi=None):
        q_, k_, v_, o_ = qb[p], kb[p], vb[p], ob[p]
        for g in range(lo // 16, (T if hi is None else hi) // 16):
            q0 = 16 * g
            qs = [q_[j, q0:q0 + 16, :] for j in range(NP)]
            ls = []
            for w in range(W):
                o = HALO + q0 - DIL * w
                acc = qs[0] * k_[0, o:o + 16, :]
                for j in range(1, NP):
                    acc = acc + qs[j] * k_[j, o:o + 16, :]
                acc = acc + pltpu.roll(acc, 64, 1)
                acc = acc + pltpu.roll(acc, 32, 1)
                if q0 < DIL * w:
                    row = lax.broadcasted_iota(i32, (16, 128), 0) + (i * T + q0 - DIL * w)
                    acc = jnp.where(row >= 0, acc, NEG)
                ls.append(acc)
            mx = ls[0]
            for l in ls[1:]:
                mx = jnp.maximum(mx, l)
            es = [jnp.exp2(l - mx) for l in ls]
            sm = es[0]
            for e in es[1:]:
                sm = sm + e
            rc = pltpu.reciprocal(sm, approx=True)
            inv = rc * (2.0 - sm * rc)
            for j in range(NP):
                acc = es[0] * v_[j, HALO + q0:HALO + q0 + 16, :]
                for w in range(1, W):
                    o = HALO + q0 - DIL * w
                    acc = acc + es[w] * v_[j, o:o + 16, :]
                o_[g * 8:g * 8 + 8, j * 128:(j + 1) * 128] = pltpu.bitcast((acc * inv).astype(bf16), u32)

    def stage_d(i, p, lo=0, hi=None):
        hi = T if hi is None else hi
        r0 = row0(i)
        wom = pltpu.bitcast(wop[...], bf16)
        hh = jnp.dot(pltpu.bitcast(ob[p][lo // 2:hi // 2, :], bf16), wom, preferred_element_type=f32)
        hb[p][lo:hi, :] = xbuf[pl.ds(r0 + lo, hi - lo), :].astype(f32) + hh

    def stage_e(i, p, carry, wrf, lo=0, hi=None):
        bval, bidx = carry
        hi = T if hi is None else hi
        r0 = row0(i)
        for c in range(lo // 16, hi // 16):
            h = hb[p][16 * c:16 * c + 16, :]
            hn = _ln(h)
            hnb[pl.ds(half0(i) + 8 * c, 8), :] = pltpu.bitcast(hn.astype(bf16), u32)
            outbuf[pl.ds(r0 + 16 * c, 16), :] = (h + hn).astype(bf16)
            r = jnp.sum(hn * wrf, axis=-1, keepdims=True)
            for g in range(2):
                rg = jnp.broadcast_to(r[8 * g:8 * g + 8, :], (8, 128))
                upd = rg > bval
                bval = jnp.where(upd, rg, bval)
                bidx = jnp.where(upd, i * T + 16 * c + 8 * g, bidx)
        return bval, bidx

    with SC('R0'):
        for j in range(NP):
            kb[1][j, T:T + HALO, :] = jnp.zeros((HALO, 128), f32)
            vb[1][j, T:T + HALO, :] = jnp.zeros((HALO, 128), f32)
        halo(0)
        wcopy(0).wait()
        prep_w(0)
    with SC('R2'):
        xcopy(0).wait()
        xcopy(1).wait()
        stage_a(0, 0)
        stage_b(0, (0,))
        stage_a(1, 1)
    with SC('R3'):
        wcopy(1).wait()
        stage_b(1, (0,))
        prep_w(1)
        stage_b(0, (1,))
    with SC('R4'):
        wcopy(2).wait()
        cp_wo.wait()
        cp_wr.wait()
        xcopy(2).wait()
        xcopy(3).start()
        xcopy(4).start()
        stage_b(1, (1,))
        prep_w(2)
        stage_b(0, (2,))
        stage_b(1, (2,))
        halo(1)
        prep_wo()
        stage_a(2, 0)
        stage_c(0, 0)
        stage_d(0, 0)
    wrf = wr[...].astype(f32).reshape(1, D)

    def step(t, par, carry):
        stage_b(par)
        halo(par)
        stage_c(t - 1, 1 - par)
        stage_d(t - 1, 1 - par)
        carry = stage_e(t - 2, par, carry, wrf)
        stage_a(t + 1, 1 - par)
        return carry

    carry = (jnp.full((8, 128), -jnp.inf, f32), jnp.zeros((8, 128), i32))

    def body(u, carry):
      with SC('iter'):
        t = 2 * u + 2
        xcopy(t + 1).wait()
        xcopy(t + 2).wait()
        xcopy(t + 3).start()

        @pl.when(u + 1 < NIT)
        def _():
            xcopy(t + 4).start()

        @pl.when(u == 0)
        def _():
            cp_wg.start()

        @pl.when(u == NIT - 1)
        def _():
            cp_wu.start()

        @pl.when(u >= 1)
        def _():
            ocopy(t - 4).start()
            ocopy(t - 3).start()
        carry = step(t, 0, carry)
        carry = step(t + 1, 1, carry)
        return carry
    carry = lax.fori_loop(0, NIT, body, carry)

    with SC('epi'):
        L = NB - 1
        xcopy(L).wait()
        cp_wd.start()
        ocopy(L - 5).start()
        ocopy(L - 4).start()
        carry = step(L - 1, 0, carry)
        ocopy(L - 3).start()
        EO = os.environ.get('EO', '2')
        if EO == '0':
            for s in range(T // BSUB):
                stage_b(1, lo=s * BSUB, hi=(s + 1) * BSUB)
            halo(1)
            stage_c(L - 1, 0)
            carry = stage_e(L - 2, 1, carry, wrf)
            ocopy(L - 2).start()
            stage_d(L - 1, 0)
            for s in range(T // SUB):
                stage_c(L, 1, s * SUB, (s + 1) * SUB)
                stage_d(L, 1, s * SUB, (s + 1) * SUB)
        elif EO == '1':
            stage_b(1, lo=0, hi=BSUB)
            halo(1)
            stage_c(L - 1, 0)
            carry = stage_e(L - 2, 1, carry, wrf)
            ocopy(L - 2).start()
            stage_c(L, 1, 0, BSUB)
            stage_d(L - 1, 0)
            stage_b(1, lo=BSUB, hi=T)
            stage_d(L, 1, 0, BSUB)
            for s in range(BSUB // SUB, T // SUB):
                stage_c(L, 1, s * SUB, (s + 1) * SUB)
                stage_d(L, 1, s * SUB, (s + 1) * SUB)
        elif EO == '2':
            stage_b(1)
            halo(1)
            stage_c(L - 1, 0)
            carry = stage_e(L - 2, 1, carry, wrf)
            ocopy(L - 2).start()
            stage_d(L - 1, 0)
            for s in range(T // SUB):
                stage_c(L, 1, s * SUB, (s + 1) * SUB)
                stage_d(L, 1, s * SUB, (s + 1) * SUB)
        carry = stage_e(L - 1, 0, carry, wrf)
        ocopy(L - 1).start()
        carry = stage_e(L, 1, carry, wrf)
        ocopy(L).start()
    bval, bidx = carry

    with SC('tail'):
        mx = jnp.max(bval, axis=0, keepdims=True)
        cand = jnp.where(bval == mx, bidx + lax.broadcasted_iota(i32, (8, 128), 0), S)
        idx = jnp.minimum(jnp.min(cand), S - 1)
        base = pl.multiple_of((idx // 16) * 16, 16)
        xs = pltpu.bitcast(hnb[pl.ds(pl.multiple_of((idx // 16) * 8, 8), 8), :], bf16)
        gate_r = jax.nn.sigmoid(mx[:, 0:1])
        cp_wg.wait()
        cp_wu.wait()
        cp_wd.wait()
        gte = jnp.dot(xs, wg[...], preferred_element_type=f32)
        up = jnp.dot(xs, wu[...], preferred_element_type=f32)
        act = (gte * jax.nn.sigmoid(gte) * up).astype(bf16)
        y = jnp.dot(act, wd[...], preferred_element_type=f32) * gate_r
        rows = lax.broadcasted_iota(i32, (16, D), 0) + base
        o16 = outbuf[pl.ds(base, 16), :].astype(f32) + jnp.where(rows == idx, y, 0.0)
        for i in range(NB):
            ocopy(i).wait()
        outbuf[pl.ds(base, 16), :] = o16.astype(bf16)
        fix = pltpu.make_async_copy(outbuf.at[pl.ds(base, 16), :], out_hbm.at[0, pl.ds(base, 16), :], sem_o.at[0])
        fix.start()
        fix.wait()


@jax.jit
def pallas_sequential_preLN__sliding_local_dilated__moe_arch_mod__prompt_kernel(A_x, A_wqkv, A_wo, B_x, B_w_r, B_w_gate, B_w_up, B_w_down):
    del B_x
    any_spec = pl.BlockSpec(memory_space=pl.ANY)
    V = pltpu.VMEM
    return pl.pallas_call(
        kernel,
        out_shape=jax.ShapeDtypeStruct((1, S, D), bf16), grid=(1,),
        in_specs=[any_spec] * 7,
        out_specs=any_spec,
        scratch_shapes=[
            V((S, D), bf16),
            V((3, D, D), bf16),
            V((D, D), bf16),
            V((NP, 320, 128), u32),
            V((960, D), u32),
            V((320, D), u32),
            V((T // 2, D), u32), V((T // 2, D), u32),
            V((NP, T, 128), f32), V((NP, T, 128), f32),
            V((NP, T + HALO, 128), f32), V((NP, T + HALO, 128), f32),
            V((NP, T + HALO, 128), f32), V((NP, T + HALO, 128), f32),
            V((T // 2, D), u32), V((T // 2, D), u32),
            V((T, D), f32), V((T, D), f32),
            V((S // 2, D), u32),
            V((S, D), bf16),
            V((D,), bf16),
            V((D, F), bf16),
            V((D, F), bf16),
            V((F, D), bf16),
            pltpu.SemaphoreType.DMA((NB,)),
            pltpu.SemaphoreType.DMA((3,)),
            pltpu.SemaphoreType.DMA((NB,)),
            pltpu.SemaphoreType.DMA((5,)),
            pltpu.SemaphoreType.REGULAR,
        ],
        compiler_params=pltpu.CompilerParams(vmem_limit_bytes=100 * 1024 * 1024),
    )(A_x, A_wqkv, A_wo, B_w_r, B_w_gate, B_w_up, B_w_down)
```

```python
import jax
import jax.numpy as jnp
from jax import lax
from jax.experimental import pallas as pl
from jax.experimental.pallas import tpu as pltpu

S, D, H, DH, W, DIL, F = 2048, 640, 32, 20, 8, 2, 1536
NP = D // 128
HALO = 16
T = 256
NB = S // T
NIT = (NB - 4) // 2
SUB = 128
EPS = 1e-5
LOG2E = 1.4426950408889634
QSCALE = DH ** -0.5 * LOG2E
NEG = -1e9 * LOG2E
f32, bf16, u32, i32 = jnp.float32, jnp.bfloat16, jnp.uint32, jnp.int32


def _ln(x):
    m = jnp.mean(x, axis=-1, keepdims=True)
    xc = x - m
    v = jnp.mean(xc * xc, axis=-1, keepdims=True)
    return xc * lax.rsqrt(v + EPS)


def _gather_rows(src, dst, dst_base, dst_col, scale=None):
    hi_mask = jnp.uint32(0xFFFF0000)
    for jp in range(NP):
        for ddl in range(2):
            dd = 2 * jp + ddl
            a = src[pl.ds(dd, 16, stride=20), :]
            b = src[pl.ds(dd + 10, 16, stride=20), :]
            if scale is None:
                lo = (a & 0xFFFF) | (b << 16)
                hi = (a >> 16) | (b & hi_mask)
            else:
                cast = lambda z: lax.bitcast_convert_type(z, f32) * scale
                lo = pltpu.pack_elementwise([cast(a << 16), cast(b << 16)], packed_dtype=bf16)
                hi = pltpu.pack_elementwise([cast(a & hi_mask), cast(b & hi_mask)], packed_dtype=bf16)
            r = dst_base + 64 * jp + 32 * ddl
            dst[r:r + 16, dst_col:dst_col + 128] = lo
            dst[r + 16:r + 32, dst_col:dst_col + 128] = hi


def kernel(x_hbm, wqkv_hbm, wo_hbm, wr_hbm, wg_hbm, wu_hbm, wd_hbm, out_hbm,
           xbuf, wraw, woraw, wt, wp, wop,
           xn0, xn1, qb0, qb1, kb0, kb1, vb0, vb1, ob0, ob1, hb0, hb1,
           hnb, outbuf, wr, wg, wu, wd,
           sem_x, sem_w, sem_o, sem_s, sem_r):
    xn, qb, kb, vb, ob, hb = (xn0, xn1), (qb0, qb1), (kb0, kb1), (vb0, vb1), (ob0, ob1), (hb0, hb1)

    def xcopy(i):
        return pltpu.make_async_copy(x_hbm.at[0, pl.ds(i * T, T), :], xbuf.at[pl.ds(i * T, T), :], sem_x.at[i])

    def ocopy(i):
        return pltpu.make_async_copy(outbuf.at[pl.ds(i * T, T), :], out_hbm.at[0, pl.ds(i * T, T), :], sem_o.at[i])

    def wcopy(m):
        return pltpu.make_async_copy(wqkv_hbm.at[:, pl.ds(m * D, D)], wraw.at[m], sem_w.at[m])

    cp_wo = pltpu.make_async_copy(wo_hbm, woraw, sem_s.at[0])
    cp_wr = pltpu.make_async_copy(wr_hbm, wr, sem_s.at[1])
    cp_wg = pltpu.make_async_copy(wg_hbm, wg, sem_s.at[2])
    cp_wu = pltpu.make_async_copy(wu_hbm, wu, sem_s.at[3])
    cp_wd = pltpu.make_async_copy(wd_hbm, wd, sem_s.at[4])

    def ordered_start(*cps):
        for cp in cps:
            cp.start()
            pl.semaphore_signal(sem_r, 1)
            pl.semaphore_wait(sem_r, 1)

    ordered_start(wcopy(0), xcopy(0), xcopy(1), wcopy(1), wcopy(2), cp_wo, cp_wr, xcopy(2))

    def row0(i):
        if isinstance(i, int):
            return i * T
        return pl.multiple_of(i * T, T)

    def half0(i):
        if isinstance(i, int):
            return i * (T // 2)
        return pl.multiple_of(i * (T // 2), T // 2)

    def transpose_chunk(m, kt):
        slab = wraw[m, kt * 128:(kt + 1) * 128, :]
        wt[kt] = pltpu.bitcast(slab.T, u32)

    def gather_w(m):
        for kt in range(NP):
            _gather_rows(wt.at[kt], wp, 320 * m, kt * 128, QSCALE if m == 0 else None)

    def prep_w(m):
        for kt in range(NP):
            transpose_chunk(m, kt)
        gather_w(m)

    def prep_wo():
        for nt in range(NP):
            wt[nt] = pltpu.bitcast(woraw[:, nt * 128:(nt + 1) * 128], u32)
        for nt in range(NP):
            _gather_rows(wt.at[nt], wop, 0, nt * 128)

    def stage_a(i, p):
        r0 = row0(i)
        for c in range(T // 16):
            x = xbuf[pl.ds(r0 + 16 * c, 16), :].astype(f32)
            xn[p][8 * c:8 * c + 8, :] = pltpu.bitcast(_ln(x).astype(bf16), u32)

    def halo(p):
        for j in range(NP):
            kb[p][j, 0:HALO, :] = kb[1 - p][j, T:T + HALO, :]
            vb[p][j, 0:HALO, :] = vb[1 - p][j, T:T + HALO, :]

    def stage_b(p, ms=(0, 1, 2), lo=0, hi=T):
        xv = pltpu.bitcast(xn[p][lo // 2:hi // 2, :], bf16)
        for m in ms:
            dst = (qb[p], kb[p], vb[p])[m]
            off = 0 if m == 0 else HALO
            wm = pltpu.bitcast(wp[320 * m:320 * (m + 1), :], bf16)
            r = lax.dot_general(xv, wm, (((1,), (1,)), ((), ())), preferred_element_type=f32)
            for j in range(NP):
                dst[j, off + lo:off + hi, :] = r[:, j * 128:(j + 1) * 128]

    def stage_c(i, p, lo=0, hi=None):
        q_, k_, v_, o_ = qb[p], kb[p], vb[p], ob[p]
        for g in range(lo // 16, (T if hi is None else hi) // 16):
            q0 = 16 * g
            qs = [q_[j, q0:q0 + 16, :] for j in range(NP)]
            ls = []
            for w in range(W):
                o = HALO + q0 - DIL * w
                acc = qs[0] * k_[0, o:o + 16, :]
                for j in range(1, NP):
                    acc = acc + qs[j] * k_[j, o:o + 16, :]
                acc = acc + pltpu.roll(acc, 64, 1)
                acc = acc + pltpu.roll(acc, 32, 1)
                if q0 < DIL * w:
                    row = lax.broadcasted_iota(i32, (16, 128), 0) + (i * T + q0 - DIL * w)
                    acc = jnp.where(row >= 0, acc, NEG)
                ls.append(acc)
            mx = ls[0]
            for l in ls[1:]:
                mx = jnp.maximum(mx, l)
            es = [jnp.exp2(l - mx) for l in ls]
            sm = es[0]
            for e in es[1:]:
                sm = sm + e
            rc = pltpu.reciprocal(sm, approx=True)
            inv = rc * (2.0 - sm * rc)
            for j in range(NP):
                acc = es[0] * v_[j, HALO + q0:HALO + q0 + 16, :]
                for w in range(1, W):
                    o = HALO + q0 - DIL * w
                    acc = acc + es[w] * v_[j, o:o + 16, :]
                o_[g * 8:g * 8 + 8, j * 128:(j + 1) * 128] = pltpu.bitcast((acc * inv).astype(bf16), u32)

    def stage_d(i, p, lo=0, hi=None):
        hi = T if hi is None else hi
        r0 = row0(i)
        wom = pltpu.bitcast(wop[...], bf16)
        hh = jnp.dot(pltpu.bitcast(ob[p][lo // 2:hi // 2, :], bf16), wom, preferred_element_type=f32)
        hb[p][lo:hi, :] = xbuf[pl.ds(r0 + lo, hi - lo), :].astype(f32) + hh

    def stage_e(i, p, carry, wrf, lo=0, hi=None):
        bval, bidx = carry
        hi = T if hi is None else hi
        r0 = row0(i)
        for c in range(lo // 16, hi // 16):
            h = hb[p][16 * c:16 * c + 16, :]
            hn = _ln(h)
            hnb[pl.ds(half0(i) + 8 * c, 8), :] = pltpu.bitcast(hn.astype(bf16), u32)
            outbuf[pl.ds(r0 + 16 * c, 16), :] = (h + hn).astype(bf16)
            r = jnp.sum(hn * wrf, axis=-1, keepdims=True)
            for g in range(2):
                rg = jnp.broadcast_to(r[8 * g:8 * g + 8, :], (8, 128))
                upd = rg > bval
                bval = jnp.where(upd, rg, bval)
                bidx = jnp.where(upd, i * T + 16 * c + 8 * g, bidx)
        return bval, bidx

    for j in range(NP):
        kb[1][j, T:T + HALO, :] = jnp.zeros((HALO, 128), f32)
        vb[1][j, T:T + HALO, :] = jnp.zeros((HALO, 128), f32)
    halo(0)
    wcopy(0).wait()
    prep_w(0)
    xcopy(0).wait()
    xcopy(1).wait()
    stage_a(0, 0)
    stage_b(0, (0,))
    stage_a(1, 1)
    wcopy(1).wait()
    stage_b(1, (0,))
    prep_w(1)
    stage_b(0, (1,))
    wcopy(2).wait()
    cp_wo.wait()
    cp_wr.wait()
    xcopy(2).wait()
    xcopy(3).start()
    xcopy(4).start()
    stage_b(1, (1,))
    prep_w(2)
    stage_b(0, (2,))
    stage_b(1, (2,))
    halo(1)
    prep_wo()
    stage_a(2, 0)
    stage_c(0, 0)
    stage_d(0, 0)
    wrf = wr[...].astype(f32).reshape(1, D)

    def step(t, par, carry):
        stage_b(par)
        halo(par)
        stage_c(t - 1, 1 - par)
        stage_d(t - 1, 1 - par)
        carry = stage_e(t - 2, par, carry, wrf)
        stage_a(t + 1, 1 - par)
        return carry

    carry = (jnp.full((8, 128), -jnp.inf, f32), jnp.zeros((8, 128), i32))

    def body(u, carry):
      t = 2 * u + 2
      xcopy(t + 1).wait()
      xcopy(t + 2).wait()
      xcopy(t + 3).start()

      @pl.when(u + 1 < NIT)
      def _():
          xcopy(t + 4).start()

      @pl.when(u == 0)
      def _():
          cp_wg.start()

      @pl.when(u == NIT - 1)
      def _():
          cp_wu.start()

      @pl.when(u >= 1)
      def _():
          ocopy(t - 4).start()
          ocopy(t - 3).start()
      carry = step(t, 0, carry)
      carry = step(t + 1, 1, carry)
      return carry
    carry = lax.fori_loop(0, NIT, body, carry)

    L = NB - 1
    xcopy(L).wait()
    cp_wd.start()
    ocopy(L - 5).start()
    ocopy(L - 4).start()
    carry = step(L - 1, 0, carry)
    ocopy(L - 3).start()
    stage_b(1)
    halo(1)
    stage_c(L - 1, 0)
    carry = stage_e(L - 2, 1, carry, wrf)
    ocopy(L - 2).start()
    stage_d(L - 1, 0)
    for s in range(T // SUB):
        stage_c(L, 1, s * SUB, (s + 1) * SUB)
        stage_d(L, 1, s * SUB, (s + 1) * SUB)
    carry = stage_e(L - 1, 0, carry, wrf)
    ocopy(L - 1).start()
    carry = stage_e(L, 1, carry, wrf)
    ocopy(L).start()
    bval, bidx = carry

    mx = jnp.max(bval, axis=0, keepdims=True)
    cand = jnp.where(bval == mx, bidx + lax.broadcasted_iota(i32, (8, 128), 0), S)
    idx = jnp.minimum(jnp.min(cand), S - 1)
    base = pl.multiple_of((idx // 16) * 16, 16)
    xs = pltpu.bitcast(hnb[pl.ds(pl.multiple_of((idx // 16) * 8, 8), 8), :], bf16)
    gate_r = jax.nn.sigmoid(mx[:, 0:1])
    cp_wg.wait()
    cp_wu.wait()
    cp_wd.wait()
    gte = jnp.dot(xs, wg[...], preferred_element_type=f32)
    up = jnp.dot(xs, wu[...], preferred_element_type=f32)
    act = (gte * jax.nn.sigmoid(gte) * up).astype(bf16)
    y = jnp.dot(act, wd[...], preferred_element_type=f32) * gate_r
    rows = lax.broadcasted_iota(i32, (16, D), 0) + base
    o16 = outbuf[pl.ds(base, 16), :].astype(f32) + jnp.where(rows == idx, y, 0.0)
    for i in range(NB):
        ocopy(i).wait()
    outbuf[pl.ds(base, 16), :] = o16.astype(bf16)
    fix = pltpu.make_async_copy(outbuf.at[pl.ds(base, 16), :], out_hbm.at[0, pl.ds(base, 16), :], sem_o.at[0])
    fix.start()
    fix.wait()


@jax.jit
def pallas_sequential_preLN__sliding_local_dilated__moe_arch_mod__prompt_kernel(A_x, A_wqkv, A_wo, B_x, B_w_r, B_w_gate, B_w_up, B_w_down):
    del B_x
    any_spec = pl.BlockSpec(memory_space=pl.ANY)
    V = pltpu.VMEM
    return pl.pallas_call(
        kernel,
        out_shape=jax.ShapeDtypeStruct((1, S, D), bf16), grid=(1,),
        in_specs=[any_spec] * 7,
        out_specs=any_spec,
        scratch_shapes=[
            V((S, D), bf16),
            V((3, D, D), bf16),
            V((D, D), bf16),
            V((NP, 320, 128), u32),
            V((960, D), u32),
            V((320, D), u32),
            V((T // 2, D), u32), V((T // 2, D), u32),
            V((NP, T, 128), f32), V((NP, T, 128), f32),
            V((NP, T + HALO, 128), f32), V((NP, T + HALO, 128), f32),
            V((NP, T + HALO, 128), f32), V((NP, T + HALO, 128), f32),
            V((T // 2, D), u32), V((T // 2, D), u32),
            V((T, D), f32), V((T, D), f32),
            V((S // 2, D), u32),
            V((S, D), bf16),
            V((D,), bf16),
            V((D, F), bf16),
            V((D, F), bf16),
            V((F, D), bf16),
            pltpu.SemaphoreType.DMA((NB,)),
            pltpu.SemaphoreType.DMA((3,)),
            pltpu.SemaphoreType.DMA((NB,)),
            pltpu.SemaphoreType.DMA((5,)),
            pltpu.SemaphoreType.REGULAR,
        ],
        compiler_params=pltpu.CompilerParams(vmem_limit_bytes=100 * 1024 * 1024),
    )(A_x, A_wqkv, A_wo, B_w_r, B_w_gate, B_w_up, B_w_down)
```
